```python
import os as _os
_os.environ.setdefault("JAX_PLATFORMS", "cpu")
import jax
import jax.numpy as jnp

def _softmax(x, axis=-1):
    return jax.nn.softmax(x, axis=axis)
def _gelu(x):
    return jax.nn.gelu(x, approximate=True)
def _silu(x):
    return jax.nn.silu(x)
def _sigmoid(x):
    return jax.nn.sigmoid(x)
def _layernorm(x, axis=-1, eps=1e-5):
    m = jnp.mean(x, axis=axis, keepdims=True)
    v = jnp.var(x, axis=axis, keepdims=True)
    return (x - m) / jnp.sqrt(v + eps)
def _scatter_add(tgt, idx, src, axis=0):
    return tgt.at[idx].add(src)
def _segment_sum(src, seg, n):
    return jax.ops.segment_sum(src, seg, n)
class _Rng:
    def __init__(self, key):
        self._k = key
    def _next(self):
        self._k, sub = jax.random.split(self._k)
        return sub
    def normal(self, shape):
        return jax.random.normal(self._next(), shape, dtype=jnp.bfloat16)
    def randint(self, lo, hi, shape):
        return jax.random.randint(self._next(), shape, lo, hi, dtype=jnp.int32)
    def uniform(self, shape, lo=0.0, hi=1.0):
        return jax.random.uniform(self._next(), shape, jnp.bfloat16, lo, hi)
    def permutation(self, n):
        return jax.random.permutation(self._next(), n)


kernel_name = 'concat_heads__gqa_block_cached__mha_block_cached__near_ridge'

def setup_inputs():
    _rng = _Rng(jax.random.key(int.from_bytes(__import__("os").urandom(4), "little")))
    _w = (lambda a: (lambda t: t.astype(jnp.bfloat16) if jnp.issubdtype(t.dtype, jnp.floating) else t)(jnp.asarray(a)))
    def _A_setup():
        B, Sq, D = 8, 112, 448
        Hq, Hkv, Sk, Dh = 16, 8, 512, 256
        assert Hq % Hkv == 0, (Hq, Hkv)
        return {
            "x": _w((lambda *s: _rng.normal(s) * 0.8)(B, Sq, D)),
            "k_cache": _w((lambda *s: _rng.normal(s) * 0.8)(B, Hkv, Sk, Dh)),
            "v_cache": _w((lambda *s: _rng.normal(s) * 0.05)(B, Hkv, Sk, Dh)),
            "wq": _w((lambda *s: _rng.normal(s) * 0.8)(D, Hq * Dh) * (D ** -0.5)),
            "wo": _w((lambda *s: _rng.normal(s) * 0.05)(Hq * Dh, D) * ((Hq * Dh) ** -0.5)),
        }
    _A_in = _A_setup()

    def _B_setup():
        B, Sq, D = 8, 112, 448
        H, Sk, Dh = 16, 512, 256
        return {
            "x": _w((lambda *s: _rng.normal(s) * 0.8)(B, Sq, D)),
            "k_cache": _w((lambda *s: _rng.normal(s) * 0.8)(B, H, Sk, Dh)),
            "v_cache": _w((lambda *s: _rng.normal(s) * 0.05)(B, H, Sk, Dh)),
            "wq": _w((lambda *s: _rng.normal(s) * 0.8)(D, H * Dh) * (D ** -0.5)),
            "wo": _w((lambda *s: _rng.normal(s) * 0.05)(H * Dh, D) * ((H * Dh) ** -0.5)),
        }
    _B_in = _B_setup()

    return {
        "A_x": _A_in["x"],
        "A_k_cache": _A_in["k_cache"],
        "A_v_cache": _A_in["v_cache"],
        "A_wq": _A_in["wq"],
        "A_wo": _A_in["wo"],
        "B_x": _B_in["x"],
        "B_k_cache": _B_in["k_cache"],
        "B_v_cache": _B_in["v_cache"],
        "B_wq": _B_in["wq"],
        "B_wo": _B_in["wo"],
    }

def reference(A_x, A_k_cache, A_v_cache, A_wq, A_wo, B_x, B_k_cache, B_v_cache, B_wq, B_wo):
    def _A_ref(x, k_cache, v_cache, wq, wo):
        B, Sq, D = x.shape
        Hq, Dh = 16, 256
        Hkv = k_cache.shape[1]
        rep = Hq // Hkv
        q = (lambda x, *d: x.transpose(*d))((x @ wq).reshape(B, Sq, Hq, Dh), 0, 2, 1, 3)
        k = jnp.repeat(k_cache, rep, axis=1)
        v = jnp.repeat(v_cache, rep, axis=1)
        scores = jnp.einsum("bhqd,bhkd->bhqk", q, k) * (Dh ** -0.5)
        p = _softmax(scores, axis=-1)
        o = jnp.einsum("bhqk,bhkd->bhqd", p, v)
        return (lambda x, *d: x.transpose(*d))(o, 0, 2, 1, 3).reshape(B, Sq, Hq * Dh) @ wo

    def _B_ref(x, k_cache, v_cache, wq, wo):
        B, Sq, D = x.shape
        H, Dh = 16, 256
        q = (lambda x, *d: x.transpose(*d))((x @ wq).reshape(B, Sq, H, Dh), 0, 2, 1, 3)
        scores = jnp.einsum("bhqd,bhkd->bhqk", q, k_cache) * (Dh ** -0.5)
        p = _softmax(scores, axis=-1)
        o = jnp.einsum("bhqk,bhkd->bhqd", p, v_cache)
        return (lambda x, *d: x.transpose(*d))(o, 0, 2, 1, 3).reshape(B, Sq, H * Dh) @ wo

    a = _A_ref(A_x, A_k_cache, A_v_cache, A_wq, A_wo)
    b = _B_ref(B_x, B_k_cache, B_v_cache, B_wq, B_wo)
    return jnp.concatenate([a, b], axis=-1)
```

```python
import jax
import jax.numpy as jnp
from jax import lax
import jax.experimental.pallas as pl
import jax.experimental.pallas.tpu as pltpu

B, SQ, D, SK, DH = 8, 112, 448, 512, 256
M = B * SQ
GW = 2 * DH
NGRP = 16
NLOOP = 14
NQ = 16
NWS = 4
HM = M // 2
NT = (((1,), (1,)), ((), ()))
f32 = jnp.float32
bf16 = jnp.bfloat16
SCALE = DH ** -0.5
S_X = 0
S_KV = 3
S_WQ = S_KV + NQ
S_WO = S_WQ + NWS
S_OUT = S_WO + NWS + 2
S_LAST = S_OUT + 3
NSEM = S_LAST + 1
LASTSLOT = (4 * 15 + 3) & (NQ - 1)


def _softmax_parts(s):
    m = jnp.max(s, axis=-1, keepdims=True)
    p = jnp.exp(s - m)
    l = jnp.sum(p, axis=-1, keepdims=True)
    r = pl.reciprocal(l, approx=True)
    r = r * (2.0 - l * r)
    return p.astype(bf16), r


def _shr(x, n):
    return x >> n if isinstance(x, int) else lax.shift_right_logical(x, n)


def _and(x, n):
    return x & n if isinstance(x, int) else lax.bitwise_and(x, n)


def _mult(x, n):
    return x if isinstance(x, int) else pl.multiple_of(x, n)


def kernel(ax_h, ak_h, av_h, awq_h, awo_h, bx_h, bk_h, bv_h, bwq_h, bwo_h, out_h,
           x_s, kv_s, wq_s, wo_s, q_s, o_s, acct_s, acctt_s, acc2_s, ob_s, sem):

    def kv_copies(br, g, qi, slot):
        b0 = 2 * qi
        s = sem.at[S_KV + slot]
        if br == 0:
            return (pltpu.make_async_copy(ak_h.at[pl.ds(b0, 2), pl.ds(g, 1)], kv_s.at[slot, :, pl.ds(0, 1)], s),
                    pltpu.make_async_copy(av_h.at[pl.ds(b0, 2), pl.ds(g, 1)], kv_s.at[slot, :, pl.ds(2, 1)], s))
        return (pltpu.make_async_copy(bk_h.at[pl.ds(b0, 2), pl.ds(2 * g, 2)], kv_s.at[slot, :, pl.ds(0, 2)], s),
                pltpu.make_async_copy(bv_h.at[pl.ds(b0, 2), pl.ds(2 * g, 2)], kv_s.at[slot, :, pl.ds(2, 2)], s))

    def per_branch(G, fn, hi=NGRP, lo=0):
        g = _and(G, 7)
        if isinstance(G, int):
            if lo <= G < hi:
                fn(G >> 3, g)
        else:
            if lo < 8:
                pl.when(G < 8)(lambda: fn(0, g))
            pl.when(jnp.logical_and(G >= max(lo, 8), G < hi))(lambda: fn(1, g))

    def kv_last_copies(u):
        s = sem.at[S_KV + LASTSLOT] if u == 0 else sem.at[S_LAST]
        return (pltpu.make_async_copy(bk_h.at[6 + u, pl.ds(14, 2)], kv_s.at[LASTSLOT, u, pl.ds(0, 2)], s),
                pltpu.make_async_copy(bv_h.at[6 + u, pl.ds(14, 2)], kv_s.at[LASTSLOT, u, pl.ds(2, 2)], s))

    def kv_start(G, half):
        for k in range(2):
            qi = 2 * half + k
            def go(br, g):
                for c in kv_copies(br, g, qi, _and(4 * G + qi, NQ - 1)):
                    c.start()
            if qi == 3 and not isinstance(G, int):
                per_branch(G, go, hi=NGRP - 1)
                @pl.when(G == NGRP - 1)
                def _():
                    for u in range(2):
                        for c in kv_last_copies(u):
                            c.start()
            else:
                per_branch(G, go)

    def kv_wait_q(G, qi):
        def go(br, g):
            for c in kv_copies(br, 0, 0, _and(4 * G + qi, NQ - 1)):
                c.wait()
        per_branch(G, go)

    def wq_copy(br, g, slot):
        src = awq_h if br == 0 else bwq_h
        return pltpu.make_async_copy(src.at[:, pl.ds(_mult(g * GW, GW), GW)], wq_s.at[slot], sem.at[S_WQ + slot])

    def wo_copy(br, g, slot):
        src = awo_h if br == 0 else bwo_h
        return pltpu.make_async_copy(src.at[:, pl.ds(_mult(g * GW, GW), GW)], wo_s.at[slot, pl.ds(64, D)], sem.at[S_WO + slot])

    def wq_start(G):
        per_branch(G, lambda br, g: wq_copy(br, g, _and(G, NWS - 1)).start())

    def wo_start(G):
        per_branch(G, lambda br, g: wo_copy(br, g, _and(G, NWS - 1)).start(), hi=NLOOP)

    def wo_tail_start(G):
        per_branch(G, lambda br, g: wo_copy(br, g, G - (NLOOP - NWS)).start(), lo=NLOOP)

    def wq_wait(G):
        wq_copy(0, 0, _and(G, NWS - 1)).wait()

    def wo_wait(G):
        wo_copy(0, 0, _and(G, NWS - 1)).wait()

    def wo_tail_wait(G):
        wo_copy(0, 0, G - (NLOOP - NWS)).wait()

    def xa_copy(h):
        return pltpu.make_async_copy(ax_h.at[pl.ds(h * HM, HM)], x_s.at[0, pl.ds(h * HM, HM)], sem.at[S_X + h])

    def xb_copy():
        return pltpu.make_async_copy(bx_h, x_s.at[1], sem.at[S_X + 2])

    def out_copy(k):
        r0, n = ((0, 6 * SQ), (6 * SQ, SQ), (7 * SQ, SQ))[k]
        return pltpu.make_async_copy(ob_s.at[pl.ds(r0, n)], out_h.at[pl.ds(r0, n)], sem.at[S_OUT + k])

    def qproj(G, r0, n):
        q = jnp.dot(x_s[_shr(G, 3), r0:r0 + n, :], wq_s[_and(G, NWS - 1)], preferred_element_type=f32)
        q_s[_and(G, 1), r0:r0 + n, :] = (q * SCALE).astype(bf16)

    def attn_unit(st, par, slot, u, r0):
        s2 = [lax.dot_general(q_s[par, pl.ds(r0, SQ), j * DH:(j + 1) * DH], kv_s[slot, u, j * st], NT,
                              preferred_element_type=f32) for j in range(2)]
        out = []
        for j in range(2):
            p, r = _softmax_parts(s2[j])
            o = jnp.dot(p, kv_s[slot, u, 2 + j * st], preferred_element_type=f32) * r
            out.append(o.astype(bf16))
        return out

    def attn_half(G, half):
        for k in range(2):
            qi = 2 * half + k
            slot = _and(4 * G + qi, NQ - 1)
            for u in range(2):
                r0 = (2 * qi + u) * SQ
                o2 = attn_unit(_shr(G, 3), _and(G, 1), slot, u, r0)
                o_s[r0:r0 + SQ, 0:DH] = o2[0]
                o_s[r0:r0 + SQ, DH:GW] = o2[1]

    def oproj_t(G):
        w = wo_s[_and(G, NWS - 1), 64:, :]
        c0 = pl.multiple_of(_shr(G, 3) * D, 64)
        for j in range(7):
            r = lax.dot_general(w, o_s[128 * j:128 * (j + 1), :], NT, preferred_element_type=f32)
            acct_s[j, pl.ds(c0, D), :] += r

    def tail_unit(G, slot, u, r0):
        o = jnp.concatenate(attn_unit(1, G & 1, slot, u, r0), axis=1)
        return lax.dot_general(o, wo_s[G - (NLOOP - NWS)], NT, preferred_element_type=f32)

    wq_start(0)
    xa_copy(0).start()
    xa_copy(1).start()
    wq_start(1)
    for G in range(2):
        kv_start(G, 0)
        wq_start(G + 2)
        kv_start(G, 1)
        wo_start(G)
    acct_s[...] = jnp.zeros(acct_s.shape, f32)
    for sl in (NWS, NWS + 1):
        wo_s[sl, 0:64, :] = jnp.zeros((64, GW), bf16)
    xa_copy(0).wait()
    wq_wait(0)
    qproj(0, 0, HM)
    xa_copy(1).wait()
    wq_wait(1)
    qproj(0, HM, HM)
    qproj(1, 0, M)
    for G in range(2, 4):
        kv_start(G, 0)
        wq_start(G + 2)
        kv_start(G, 1)
        wo_start(G)
    xb_copy().start()

    def body(G, carry):
        kv_wait_q(G, 0)
        kv_wait_q(G, 1)
        wq_wait(G + 2)
        pl.when(G == 6)(lambda: xb_copy().wait())
        attn_half(G, 0)
        qproj(G + 2, 0, HM)
        kv_start(G + 4, 0)
        kv_wait_q(G, 2)
        kv_wait_q(G, 3)
        wo_wait(G)
        attn_half(G, 1)
        qproj(G + 2, HM, HM)
        oproj_t(G)
        wq_start(G + 6)
        kv_start(G + 4, 1)
        wo_start(G + 4)
        wo_tail_start(G + 5)
        return carry

    lax.fori_loop(0, NLOOP, body, 0)

    def tail1(h, carry):
        G = 14
        for k in range(2):
            for c in kv_copies(1, 0, 0, _and(4 * G + 2 * h + k, NQ - 1)):
                c.wait()
        pl.when(h == 0)(lambda: wo_tail_wait(G))
        for k in range(4):
            j = jnp.minimum(4 * h + k, 6)
            acctt_s[pl.ds(pl.multiple_of(j * 128, 128), 128), :] = acct_s[j].T
        for k in range(2):
            slot = _and(4 * G + 2 * h + k, NQ - 1)
            for u in range(2):
                r0 = pl.multiple_of((4 * h + 2 * k + u) * SQ, 16)
                acc2_s[pl.ds(r0, SQ), :] = tail_unit(G, slot, u, r0)
        return carry

    lax.fori_loop(0, 2, tail1, 0)

    def final_unit(slot, u, r0):
        r = tail_unit(15, slot, u, r0)
        ob_s[pl.ds(r0, SQ), 0:384] = acctt_s[pl.ds(r0, SQ), 0:384].astype(bf16)
        ob_s[pl.ds(r0, SQ), 384:896] = (acctt_s[pl.ds(r0, SQ), 384:896] + acc2_s[pl.ds(r0, SQ), :] + r).astype(bf16)

    def tail2(qi, carry):
        G = 15
        slot = _and(4 * G + qi, NQ - 1)
        for c in kv_copies(1, 0, 0, slot):
            c.wait()
        pl.when(qi == 0)(lambda: wo_tail_wait(G))
        for u in range(2):
            final_unit(slot, u, pl.multiple_of((2 * qi + u) * SQ, 16))
        return carry

    lax.fori_loop(0, 3, tail2, 0)
    for c in kv_last_copies(0):
        c.wait()
    out_copy(0).start()
    final_unit(LASTSLOT, 0, 6 * SQ)
    out_copy(1).start()
    for c in kv_last_copies(1):
        c.wait()
    final_unit(LASTSLOT, 1, 7 * SQ)
    out_copy(2).start()
    for k in range(3):
        out_copy(k).wait()


@jax.jit
def pallas_concat_heads__gqa_block_cached__mha_block_cached__near_ridge_kernel(A_x, A_k_cache, A_v_cache, A_wq, A_wo, B_x, B_k_cache, B_v_cache, B_wq, B_wo):
    hbm = pl.BlockSpec(memory_space=pl.ANY)
    out = pl.pallas_call(
        kernel,
        in_specs=[hbm] * 10,
        out_specs=hbm,
        out_shape=jax.ShapeDtypeStruct((M, 2 * D), bf16),
        scratch_shapes=[
            pltpu.VMEM((2, M, D), bf16),
            pltpu.VMEM((NQ, 2, 4, SK, DH), bf16),
            pltpu.VMEM((NWS, D, GW), bf16),
            pltpu.VMEM((NWS + 2, 512, GW), bf16),
            pltpu.VMEM((2, M, GW), bf16),
            pltpu.VMEM((M, GW), bf16),
            pltpu.VMEM((7, 2 * D, 128), f32),
            pltpu.VMEM((M, 2 * D), f32),
            pltpu.VMEM((M, 512), f32),
            pltpu.VMEM((M, 2 * D), bf16),
            pltpu.SemaphoreType.DMA((NSEM,)),
        ],
        compiler_params=pltpu.CompilerParams(vmem_limit_bytes=100 * 1024 * 1024, disable_bounds_checks=True),
    )(A_x.reshape(M, D), A_k_cache, A_v_cache, A_wq, A_wo.T, B_x.reshape(M, D), B_k_cache, B_v_cache, B_wq, B_wo.T)
    return out.reshape(B, SQ, 2 * D)
```

```python
import jax
import jax.numpy as jnp
from jax import lax
import jax.experimental.pallas as pl
import jax.experimental.pallas.tpu as pltpu

B, SQ, D, SK, DH = 8, 112, 448, 512, 256
M = B * SQ
GW = 2 * DH
NGRP = 16
NLOOP = 14
NWS = 4
HM = M // 2
NT = (((1,), (1,)), ((), ()))
f32 = jnp.float32
bf16 = jnp.bfloat16
SCALE = DH ** -0.5
P0 = 0
P1 = 1
R0 = 128
RB = SK - R0
LA = 5
H13 = 0
FULLHI = 13 if H13 else 14
QSPLIT = 2
OSPLIT = 2
OPG = ((0,), (1,), (2,), (3,))
T2 = ((0, 4), (4, 3), (7, 1))
S_X = 0
S_B = 3
S_W0 = S_B + 64
S_LAST = S_W0 + 5
S_OUT = S_LAST + 1
NSEM = S_OUT + 3


def _softmax_parts(s):
    m = jnp.max(s, axis=-1, keepdims=True)
    p = jnp.exp(s - m)
    l = jnp.sum(p, axis=-1, keepdims=True)
    r = pl.reciprocal(l, approx=True)
    r = r * (2.0 - l * r)
    return p.astype(bf16), r


def _shr(x, n):
    return x >> n if isinstance(x, int) else lax.shift_right_logical(x, n)


def _and(x, n):
    return x & n if isinstance(x, int) else lax.bitwise_and(x, n)


def _mult(x, n):
    return x if isinstance(x, int) else pl.multiple_of(x, n)


def _when(cond, fn):
    if isinstance(cond, bool):
        if cond:
            fn()
    else:
        pl.when(cond)(fn)


def _rng(G, lo, hi):
    if isinstance(G, int):
        return lo <= G < hi
    return jnp.logical_and(G >= lo, G < hi)


def kernel(ax_h, ak_h, av_h, awq_h, awo_h, bx_h, bk_h, bv_h, bwq_h, bwo_h, out_h,
           x_s, k_s, v_s, wq_s, wo_s, q_s, o_s, acct_s, acc2_s, ob_s,
           sem, ksem, vsem, wqsem, wosem):
    cp = pltpu.make_async_copy
    KV = ((ak_h, bk_h, k_s, ksem), (av_h, bv_h, v_s, vsem))

    def per_branch(G, fn, lo=0, hi=NGRP):
        g = _and(G, 7)
        _when(_rng(G, lo, 8), lambda: fn(0, g))
        _when(_rng(G, max(lo, 8), hi), lambda: fn(1, g))

    def piece_start(kind, G, u, j):
        a_h, b_h, buf, ps = KV[kind]
        def go(br, g):
            if br == 0:
                h = R0 // 2
                c = cp(a_h.at[u, g, pl.ds(j * h, h)], buf.at[g, u, pl.ds(j * h, h)], ps.at[_and(G, 1)])
            else:
                r = j * (2 * SK - R0)
                c = cp(b_h.at[u, pl.ds(_mult(2 * SK * g + r, 16), R0)], buf.at[g, u, pl.ds(r, R0)], ps.at[_and(G, 1)])
            c.start(priority=P0)
        per_branch(G, go, lo=2, hi=15)

    def piece_wait(G, lo=2, hi=15):
        def go(br, g):
            for kind in range(2):
                buf, ps = KV[kind][2], KV[kind][3]
                dst = buf.at[g, :, pl.ds(0, (1 + br) * R0)]
                cp(dst, dst, ps.at[_and(G, 1)]).wait()
        per_branch(G, go, lo=lo, hi=hi)

    def bulk(kind, br, g, b0, nb, r0, s):
        a_h, b_h, buf, _ = KV[kind]
        if br == 0:
            return cp(a_h.at[pl.ds(b0, nb), g, pl.ds(r0, SK - r0)],
                      buf.at[g, pl.ds(b0, nb), pl.ds(r0, SK - r0)], s)
        n = 2 * (SK - r0)
        return cp(b_h.at[pl.ds(b0, nb), pl.ds(_mult(2 * SK * g + r0, 16), n)],
                  buf.at[g, pl.ds(b0, nb), pl.ds(r0, n)], s)

    def last_copies(k):
        b0, nb = T2[k]
        return [bulk(kind, 1, 7, b0, nb, 0, sem.at[S_B + 60 + k]) for kind in range(2)]

    def refill(G):
        Gn = G + LA
        g = _and(Gn, 7)
        def whole():
            for kind in range(2):
                bulk(kind, 1, g, 0, 8, R0, sem.at[S_B + 4 * Gn]).start(priority=P1)
        def by_half():
            for h in range(2):
                for kind in range(2):
                    bulk(kind, 1, g, 4 * h, 4, R0, sem.at[S_B + 4 * Gn + h]).start(priority=P1)
        def g15():
            for k in range(3):
                for c in last_copies(k):
                    c.start(priority=P1)
        pl.when(_rng(Gn, 8, FULLHI))(whole)
        pl.when(_rng(Gn, FULLHI, 15))(by_half)
        pl.when(Gn == 15)(g15)

    def bulk_wait_h(G, h):
        for kind in range(2):
            bulk(kind, 1, 0, 0, 4, R0, sem.at[S_B + 4 * G + h]).wait()

    def bulk_wait_full_br(br, G):
        for kind in range(2):
            bulk(kind, br, 0, 0, 8, R0, sem.at[S_B + 4 * G]).wait()

    def bulk_wait_q(G, qi, r0):
        for kind in range(2):
            bulk(kind, 1, 0, 0, 2, r0, sem.at[S_B + 4 * G + qi]).wait()

    def start_copies(G, h):
        return [bulk(kind, 0, G, 4 * h, 4, 0, sem.at[S_B + 4 * G + h]) for kind in range(2)]

    def wq_piece(br, g, slot, r0, n, s):
        src = awq_h if br == 0 else bwq_h
        return cp(src.at[pl.ds(r0, n), pl.ds(_mult(g * GW, GW), GW)], wq_s.at[slot, pl.ds(r0, n)], s)

    def wo_piece(br, g, slot, r0, n, s):
        src = awo_h if br == 0 else bwo_h
        return cp(src.at[pl.ds(r0, n), pl.ds(_mult(g * GW, GW), GW)], wo_s.at[slot, pl.ds(64 + r0, n)], s)

    def wq_piece_start(G, k, n):
        sl = _and(G, NWS - 1)
        rows = D // n
        per_branch(G, lambda br, g: wq_piece(br, g, sl, rows * k, rows, wqsem.at[sl]).start(priority=P0))

    def wo_piece_start(G, k, n):
        sl = _and(G, NWS - 1)
        rows = D // n
        per_branch(G, lambda br, g: wo_piece(br, g, sl, rows * k, rows, wosem.at[sl]).start(priority=P0))

    def wq_wait(G):
        sl = _and(G, NWS - 1)
        wq_piece(0, 0, sl, 0, D, wqsem.at[sl]).wait()

    def wo_wait(G):
        sl = _and(G, NWS - 1)
        wo_piece(0, 0, sl, 0, D, wosem.at[sl]).wait()

    def xa_copy(h):
        return cp(ax_h.at[pl.ds(h * HM, HM)], x_s.at[0, pl.ds(h * HM, HM)], sem.at[S_X + h])

    def xb_copy():
        return cp(bx_h, x_s.at[1], sem.at[S_X + 2])

    def out_copy(k):
        r0, n = T2[k][0] * SQ, T2[k][1] * SQ
        return cp(ob_s.at[pl.ds(r0, n)], out_h.at[pl.ds(r0, n)], sem.at[S_OUT + k])

    def qproj(G, r0, n, before=None):
        x = x_s[_shr(G, 3), r0:r0 + n, :]
        for k in range(4):
            if before is not None:
                before(k)
            q = jnp.dot(x, wq_s[_and(G, NWS - 1), :, 128 * k:128 * (k + 1)], preferred_element_type=f32)
            q_s[_and(G, 1), r0:r0 + n, 128 * k:128 * (k + 1)] = (q * SCALE).astype(bf16)

    def attn_unit(st, par, slot, u, r0, before=None):
        s2 = []
        for j in range(2):
            if before is not None:
                before(0, j)
            s2.append(lax.dot_general(q_s[par, pl.ds(r0, SQ), j * DH:(j + 1) * DH], k_s[slot, u, pl.ds(_mult(j * st * SK, SK), SK)], NT,
                                      preferred_element_type=f32))
        out = []
        for j in range(2):
            p, r = _softmax_parts(s2[j])
            if before is not None:
                before(1, j)
            o = jnp.dot(p, v_s[slot, u, pl.ds(_mult(j * st * SK, SK), SK)], preferred_element_type=f32) * r
            out.append(o.astype(bf16))
        return out

    def attn_units(G, u0, u1, do_refill=False):
        for u in range(u0, u1):
            r0 = u * SQ
            def before(kind, j):
                if u == u0 and kind == 0:
                    if j == 1:
                        piece_start(0, G + 1, u, 0)
                        piece_start(0, G + 1, u, 1)
                else:
                    piece_start(kind, G + 1, u, j)
            o2 = attn_unit(_shr(G, 3), _and(G, 1), _and(G, 7), u, r0, before=before)
            o_s[r0:r0 + SQ, 0:DH] = o2[0]
            o_s[r0:r0 + SQ, DH:GW] = o2[1]
            if u == 1 and do_refill:
                refill(G)

    def oproj_t(G):
        c0 = _shr(G, 3) * D
        rows = D // OSPLIT
        for j in range(7):
            for t in range(OSPLIT):
                r = lax.dot_general(wo_s[_and(G, NWS - 1), 64 + rows * t:64 + rows * (t + 1), :],
                                    o_s[128 * j:128 * (j + 1), :], NT, preferred_element_type=f32)
                acct_s[j, pl.ds(_mult(c0 + rows * t, 32), rows), :] += r
                wo_piece_start(G + 2, j * OSPLIT + t, 7 * OSPLIT)

    def a_transpose(j):
        ob_s[pl.ds(_mult(j * 128, 128), 128), 0:384] = acct_s[j, 0:384, :].T.astype(bf16)

    def tail_unit(G, u, r0):
        o = jnp.concatenate(attn_unit(1, G & 1, G & 7, u, r0), axis=1)
        return lax.dot_general(o, wo_s[G & (NWS - 1)], NT, preferred_element_type=f32)

    w0 = [wq_piece(0, 0, 0, 0, D, sem.at[S_W0]), wq_piece(0, 1, 1, 0, D, sem.at[S_W0 + 1]),
          wq_piece(0, 2, 2, 0, D, sem.at[S_W0 + 2])]

    def wo01(G):
        return wo_piece(0, G, G, 0, D, sem.at[S_W0 + 3 + G])

    first = [w0[0], xa_copy(0), xa_copy(1), w0[1]]
    first += start_copies(0, 0) + [w0[2]] + start_copies(0, 1) + [wo01(0)]
    first += start_copies(1, 0) + start_copies(1, 1) + [wo01(1)]
    for G in range(2, 8):
        if G == 5:
            first.append(xb_copy())
        first += [bulk(kind, 0, G, 0, 8, R0, sem.at[S_B + 4 * G]) for kind in range(2)]
    for c in first:
        c.start(priority=P1)
    acct_s[...] = jnp.zeros(acct_s.shape, f32)
    for sl in (2, 3):
        wo_s[sl, 0:64, :] = jnp.zeros((64, GW), bf16)
    xa_copy(0).wait()
    w0[0].wait()
    qproj(0, 0, HM)
    xa_copy(1).wait()
    w0[1].wait()
    qproj(0, HM, HM)
    qproj(1, 0, M)
    for c in start_copies(0, 0):
        c.wait()
    w0[2].wait()

    def wait_top(Gn):
        @pl.when(Gn == 1)
        def _():
            for c in start_copies(1, 0):
                c.wait()
        piece_wait(Gn)
        _when(_rng(Gn, 2, 8), lambda: bulk_wait_full_br(0, Gn))
        _when(_rng(Gn, 8, FULLHI), lambda: bulk_wait_full_br(1, Gn))
        pl.when(Gn >= FULLHI)(lambda: bulk_wait_h(Gn, 0))
        pl.when(Gn < NLOOP)(lambda: wq_wait(Gn + 2))
        pl.when(jnp.logical_and(Gn >= 2, Gn != (13 if H13 else 0)))(lambda: wo_wait(Gn))
        pl.when(Gn == 6)(lambda: xb_copy().wait())

    def halves(G):
        attn_units(G, 0, 4)
        qproj(G + 2, 0, HM, before=lambda k: wq_piece_start(G + 3, k, 8))
        for c in start_copies(G, 1):
            c.wait()
        wo01(G).wait()
        attn_units(G, 4, 8)
        qproj(G + 2, HM, HM, before=lambda k: wq_piece_start(G + 3, 4 + k, 8))
        oproj_t(G)
        wait_top(G + 1)

    def full(G):
        a_transpose(jnp.clip(G - 8, 0, 6))
        attn_units(G, 0, 8, do_refill=True)
        n = M // QSPLIT
        for t in range(QSPLIT):
            qproj(G + 2, n * t, n, before=lambda k: wq_piece_start(G + 3, 4 * t + k, 4 * QSPLIT))
        oproj_t(G)
        wait_top(G + 1)

    def body_h(G, carry):
        halves(G)
        return carry

    def body_f(G, carry):
        full(G)
        return carry

    lax.fori_loop(0, 2, body_h, 0)
    lax.fori_loop(2, NLOOP, body_f, 0)

    for h in range(2):
        tt = jnp.concatenate([acct_s[3 * h + k, 384:, :].T for k in range(4)], axis=0)
        os_ = [jnp.concatenate(attn_unit(1, 0, 6, 4 * h + k, (4 * h + k) * SQ), axis=1) for k in range(4)]
        for grp in OPG:
            o = jnp.concatenate([os_[k] for k in grp], axis=0)
            r = lax.dot_general(o, wo_s[14 & (NWS - 1)], NT, preferred_element_type=f32)
            n = len(grp) * SQ
            r0 = (4 * h + grp[0]) * SQ
            t0 = 64 * h + grp[0] * SQ
            acc2_s[r0:r0 + n, :] = tt[t0:t0 + n] + r
        if h == 0:
            bulk_wait_h(14, 1)
        else:
            for c in last_copies(0):
                c.wait()
            wo_wait(15)

    def final_unit(u, r0):
        r = tail_unit(15, u, r0)
        ob_s[pl.ds(r0, SQ), 384:896] = (acc2_s[pl.ds(r0, SQ), :] + r).astype(bf16)

    a_transpose(6)
    for k in range(3):
        b0, nb = T2[k]
        os_ = [jnp.concatenate(attn_unit(1, 1, 7, u, u * SQ), axis=1) for u in range(b0, b0 + nb)]
        for u in range(b0, b0 + nb):
            r = lax.dot_general(os_[u - b0], wo_s[15 & (NWS - 1)], NT, preferred_element_type=f32)
            ob_s[u * SQ:(u + 1) * SQ, 384:896] = (acc2_s[u * SQ:(u + 1) * SQ, :] + r).astype(bf16)
        out_copy(k).start()
        if k < 2:
            for c in last_copies(k + 1):
                c.wait()
        else:
            for j in range(3):
                out_copy(j).wait()


@jax.jit
def pallas_concat_heads__gqa_block_cached__mha_block_cached__near_ridge_kernel(A_x, A_k_cache, A_v_cache, A_wq, A_wo, B_x, B_k_cache, B_v_cache, B_wq, B_wo):
    hbm = pl.BlockSpec(memory_space=pl.ANY)
    out = pl.pallas_call(
        kernel,
        in_specs=[hbm] * 10,
        out_specs=hbm,
        out_shape=jax.ShapeDtypeStruct((M, 2 * D), bf16),
        scratch_shapes=[
            pltpu.VMEM((2, M, D), bf16),
            pltpu.VMEM((8, B, 2 * SK, DH), bf16),
            pltpu.VMEM((8, B, 2 * SK, DH), bf16),
            pltpu.VMEM((NWS, D, GW), bf16),
            pltpu.VMEM((NWS, 512, GW), bf16),
            pltpu.VMEM((2, M, GW), bf16),
            pltpu.VMEM((M, GW), bf16),
            pltpu.VMEM((7, 2 * D, 128), f32),
            pltpu.VMEM((M, 512), f32),
            pltpu.VMEM((M, 2 * D), bf16),
            pltpu.SemaphoreType.DMA((NSEM,)),
            pltpu.SemaphoreType.DMA((2,)),
            pltpu.SemaphoreType.DMA((2,)),
            pltpu.SemaphoreType.DMA((NWS,)),
            pltpu.SemaphoreType.DMA((NWS,)),
        ],
        compiler_params=pltpu.CompilerParams(vmem_limit_bytes=110 * 1024 * 1024, disable_bounds_checks=True,
                                             disable_semaphore_checks=True),
    )(A_x.reshape(M, D), A_k_cache, A_v_cache, A_wq, A_wo.T, B_x.reshape(M, D), B_k_cache.reshape(B, 16 * SK, DH), B_v_cache.reshape(B, 16 * SK, DH), B_wq, B_wo.T)
    return out.reshape(B, SQ, 2 * D)
```

```python
import jax
import jax.numpy as jnp
from jax import lax
import jax.experimental.pallas as pl
import jax.experimental.pallas.tpu as pltpu

B, SQ, D, SK, DH = 8, 112, 448, 512, 256
M = B * SQ
GW = 2 * DH
NGRP = 16
NLOOP = 14
NWS = 4
HM = M // 2
NT = (((1,), (1,)), ((), ()))
f32 = jnp.float32
bf16 = jnp.bfloat16
SCALE = DH ** -0.5
P0 = 0
P1 = 1
QFIRST = 1
HFIRST = 1
R0 = 160
RB = SK - R0
LA = 5
H13 = 0
FULLHI = 13 if H13 else 14
QSPLIT = 2
OSPLIT = 2
OPG = ((0,), (1,), (2,), (3,))
T2 = ((0, 4), (4, 3), (7, 1))
S_X = 0
S_B = 3
S_W0 = S_B + 64
S_LAST = S_W0 + 5
S_OUT = S_LAST + 1
NSEM = S_OUT + 4


def _softmax_parts(s):
    m = jnp.max(s, axis=-1, keepdims=True)
    p = jnp.exp(s - m)
    l = jnp.sum(p, axis=-1, keepdims=True)
    r = pl.reciprocal(l, approx=True)
    r = r * (2.0 - l * r)
    return p.astype(bf16), r


def _shr(x, n):
    return x >> n if isinstance(x, int) else lax.shift_right_logical(x, n)


def _and(x, n):
    return x & n if isinstance(x, int) else lax.bitwise_and(x, n)


def _mult(x, n):
    return x if isinstance(x, int) else pl.multiple_of(x, n)


def _when(cond, fn):
    if isinstance(cond, bool):
        if cond:
            fn()
    else:
        pl.when(cond)(fn)


def _rng(G, lo, hi):
    if isinstance(G, int):
        return lo <= G < hi
    return jnp.logical_and(G >= lo, G < hi)


def kernel(ax_h, ak_h, av_h, awq_h, awo_h, bx_h, bk_h, bv_h, bwq_h, bwo_h, out_h,
           x_s, k_s, v_s, wq_s, wo_s, q_s, o_s, acct_s, acc2_s, ob_s,
           sem, ksem, vsem, wqsem, wosem):
    cp = pltpu.make_async_copy
    KV = ((ak_h, bk_h, k_s, ksem), (av_h, bv_h, v_s, vsem))

    def per_branch(G, fn, lo=0, hi=NGRP):
        g = _and(G, 7)
        _when(_rng(G, lo, 8), lambda: fn(0, g))
        _when(_rng(G, max(lo, 8), hi), lambda: fn(1, g))

    def piece_start(kind, G, u, j):
        a_h, b_h, buf, ps = KV[kind]
        def go(br, g):
            if br == 0:
                h = R0 // 2
                c = cp(a_h.at[u, g, pl.ds(j * h, h)], buf.at[g, u, pl.ds(j * h, h)], ps.at[_and(G, 1)])
            else:
                r = j * (2 * SK - R0)
                c = cp(b_h.at[u, pl.ds(_mult(2 * SK * g + r, 16), R0)], buf.at[g, u, pl.ds(r, R0)], ps.at[_and(G, 1)])
            c.start(priority=P0)
        per_branch(G, go, lo=2, hi=15)

    def piece_wait(G, lo=2, hi=15):
        def go(br, g):
            for kind in range(2):
                buf, ps = KV[kind][2], KV[kind][3]
                for r in ((0,), (0, 2 * SK - R0))[br]:
                    dst = buf.at[g, :, pl.ds(r, R0)]
                    cp(dst, dst, ps.at[_and(G, 1)]).wait()
        per_branch(G, go, lo=lo, hi=hi)

    def piece15(kind, u, j, par):
        buf, ps = KV[kind][2], KV[kind][3]
        r = j * (2 * SK - R0)
        return cp(KV[kind][1].at[u, pl.ds(2 * SK * 7 + r, R0)], buf.at[7, u, pl.ds(r, R0)], ps.at[par])

    def piece15_wait(k):
        b0, nb = T2[k]
        for kind in range(2):
            for u in range(b0, b0 + nb):
                for j in range(2):
                    piece15(kind, u, j, (k + 1) % 2).wait()

    def pins15(k, first):
        b0, nb = T2[k]
        def make(u):
            i = u - first
            if i >= nb:
                return None
            def before(kind, j):
                if i == 0 and kind == 0:
                    if j == 1:
                        piece15(0, b0, 0, (k + 1) % 2).start(priority=P0)
                        piece15(0, b0, 1, (k + 1) % 2).start(priority=P0)
                else:
                    piece15(kind, b0 + i, j, (k + 1) % 2).start(priority=P0)
            return before
        return make

    def bulk(kind, br, g, b0, nb, r0, s):
        a_h, b_h, buf, _ = KV[kind]
        if br == 0:
            return cp(a_h.at[pl.ds(b0, nb), g, pl.ds(r0, SK - r0)],
                      buf.at[g, pl.ds(b0, nb), pl.ds(r0, SK - r0)], s)
        n = 2 * (SK - r0)
        return cp(b_h.at[pl.ds(b0, nb), pl.ds(_mult(2 * SK * g + r0, 16), n)],
                  buf.at[g, pl.ds(b0, nb), pl.ds(r0, n)], s)

    def last_copies(k):
        b0, nb = T2[k]
        return [bulk(kind, 1, 7, b0, nb, R0, sem.at[S_B + 60 + k]) for kind in range(2)]

    def refill(G):
        Gn = G + LA
        g = _and(Gn, 7)
        def whole():
            for kind in range(2):
                bulk(kind, 1, g, 0, 8, R0, sem.at[S_B + 4 * Gn]).start(priority=P1)
        def by_half():
            for h in range(2):
                for kind in range(2):
                    bulk(kind, 1, g, 4 * h, 4, R0, sem.at[S_B + 4 * Gn + h]).start(priority=P1)
        def g15():
            for k in range(3):
                for c in last_copies(k):
                    c.start(priority=P1)
        pl.when(_rng(Gn, 8, FULLHI))(whole)
        pl.when(_rng(Gn, FULLHI, 15))(by_half)
        pl.when(Gn == 15)(g15)

    def bulk_wait_h(G, h):
        for kind in range(2):
            bulk(kind, 1, _and(G, 7), 4 * h, 4, R0, sem.at[S_B + 4 * G + h]).wait()

    def bulk_wait_full_br(br, G):
        for kind in range(2):
            bulk(kind, br, _and(G, 7), 0, 8, R0, sem.at[S_B + 4 * G]).wait()

    def start_copies(G, h):
        return [bulk(kind, 0, G, 4 * h, 4, 0, sem.at[S_B + 4 * G + h]) for kind in range(2)]

    def wq_piece(br, g, slot, r0, n, s):
        src = awq_h if br == 0 else bwq_h
        return cp(src.at[pl.ds(r0, n), pl.ds(_mult(g * GW, GW), GW)], wq_s.at[slot, pl.ds(r0, n)], s)

    def wo_piece(br, g, slot, r0, n, s):
        src = awo_h if br == 0 else bwo_h
        return cp(src.at[pl.ds(r0, n), pl.ds(_mult(g * GW, GW), GW)], wo_s.at[slot, pl.ds(64 + r0, n)], s)

    def wq_piece_start(G, k, n):
        sl = _and(G, NWS - 1)
        rows = D // n
        per_branch(G, lambda br, g: wq_piece(br, g, sl, rows * k, rows, wqsem.at[sl]).start(priority=P0))

    def wo_piece_start(G, k, n):
        sl = _and(G, NWS - 1)
        rows = D // n
        per_branch(G, lambda br, g: wo_piece(br, g, sl, rows * k, rows, wosem.at[sl]).start(priority=P0))

    def wq_wait(G):
        sl = _and(G, NWS - 1)
        wq_piece(0, 0, sl, 0, D, wqsem.at[sl]).wait()

    def wo_wait(G):
        sl = _and(G, NWS - 1)
        wo_piece(0, 0, sl, 0, D, wosem.at[sl]).wait()

    def xa_copy(h):
        return cp(ax_h.at[pl.ds(h * HM, HM)], x_s.at[0, pl.ds(h * HM, HM)], sem.at[S_X + h])

    def xb_copy():
        return cp(bx_h, x_s.at[1], sem.at[S_X + 2])

    def out_copy(k):
        if k == 3:
            return cp(ob_s.at[pl.ds(7 * SQ, SQ), pl.ds(0, 384)], out_h.at[pl.ds(7 * SQ, SQ), pl.ds(0, 384)], sem.at[S_OUT + 3])
        r0, n = T2[k][0] * SQ, T2[k][1] * SQ
        if k == 2:
            return cp(ob_s.at[pl.ds(r0, n), pl.ds(384, 512)], out_h.at[pl.ds(r0, n), pl.ds(384, 512)], sem.at[S_OUT + k])
        return cp(ob_s.at[pl.ds(r0, n)], out_h.at[pl.ds(r0, n)], sem.at[S_OUT + k])

    def qproj(G, r0, n, before=None):
        x = x_s[_shr(G, 3), r0:r0 + n, :]
        for k in range(4):
            if before is not None:
                before(k)
            q = jnp.dot(x, wq_s[_and(G, NWS - 1), :, 128 * k:128 * (k + 1)], preferred_element_type=f32)
            q_s[_and(G, 3), r0:r0 + n, 128 * k:128 * (k + 1)] = (q * SCALE).astype(bf16)

    def attn_unit(st, par, slot, u, r0, before=None):
        s2 = []
        for j in range(2):
            if before is not None:
                before(0, j)
            s2.append(lax.dot_general(q_s[par, pl.ds(r0, SQ), j * DH:(j + 1) * DH], k_s[slot, u, pl.ds(_mult(j * st * SK, SK), SK)], NT,
                                      preferred_element_type=f32))
        out = []
        for j in range(2):
            p, r = _softmax_parts(s2[j])
            if before is not None:
                before(1, j)
            o = jnp.dot(p, v_s[slot, u, pl.ds(_mult(j * st * SK, SK), SK)], preferred_element_type=f32) * r
            out.append(o.astype(bf16))
        return out

    def attn_units(G, u0, u1, do_refill=False):
        for u in range(u0, u1):
            r0 = u * SQ
            def before(kind, j):
                if u == u0 and kind == 0:
                    if j == 1:
                        piece_start(0, G + 1, u, 0)
                        piece_start(0, G + 1, u, 1)
                else:
                    piece_start(kind, G + 1, u, j)
            o2 = attn_unit(_shr(G, 3), _and(G, 3), _and(G, 7), u, r0, before=before)
            o_s[r0:r0 + SQ, 0:DH] = o2[0]
            o_s[r0:r0 + SQ, DH:GW] = o2[1]
            if u == 1 and do_refill:
                refill(G)

    def oproj_t(G):
        c0 = _shr(G, 3) * D
        rows = D // OSPLIT
        for j in range(7):
            for t in range(OSPLIT):
                r = lax.dot_general(wo_s[_and(G, NWS - 1), 64 + rows * t:64 + rows * (t + 1), :],
                                    o_s[128 * j:128 * (j + 1), :], NT, preferred_element_type=f32)
                acct_s[j, pl.ds(_mult(c0 + rows * t, 32), rows), :] += r
                wo_piece_start(G + 2, j * OSPLIT + t, 7 * OSPLIT)

    def a_transpose(j):
        ob_s[pl.ds(_mult(j * 128, 128), 128), 0:384] = acct_s[j, 0:384, :].T.astype(bf16)

    w0 = [wq_piece(0, 0, 0, 0, D, sem.at[S_W0]), wq_piece(0, 1, 1, 0, D, sem.at[S_W0 + 1]),
          wq_piece(0, 2, 2, 0, D, sem.at[S_W0 + 2])]

    def wo01(G):
        return wo_piece(0, G, G, 0, D, sem.at[S_W0 + 3 + G])

    first = [w0[0], xa_copy(0), xa_copy(1), w0[1]]
    first += start_copies(0, 0) + [w0[2]] + start_copies(0, 1) + [wo01(0)]
    first += start_copies(1, 0) + start_copies(1, 1) + [wo01(1)]
    for G in range(2, 8):
        if G == 5:
            first.append(xb_copy())
        first += [bulk(kind, 0, G, 0, 8, R0, sem.at[S_B + 4 * G]) for kind in range(2)]
    for c in first:
        c.start(priority=P1)
    acct_s[...] = jnp.zeros(acct_s.shape, f32)
    wo_s[3, 0:64, :] = jnp.zeros((64, GW), bf16)
    xa_copy(0).wait()
    w0[0].wait()
    qproj(0, 0, HM)
    xa_copy(1).wait()
    w0[1].wait()
    qproj(0, HM, HM)
    qproj(1, 0, M)
    for c in start_copies(0, 0):
        c.wait()
    w0[2].wait()

    def wait_top(Gn):
        @pl.when(Gn == 1)
        def _():
            for c in start_copies(1, 0):
                c.wait()
        piece_wait(Gn)
        _when(_rng(Gn, 2, 8), lambda: bulk_wait_full_br(0, Gn))
        _when(_rng(Gn, 8, FULLHI), lambda: bulk_wait_full_br(1, Gn))
        pl.when(Gn >= FULLHI)(lambda: bulk_wait_h(Gn, 0))
        pl.when(Gn < NLOOP)(lambda: wq_wait(Gn + 2))
        pl.when(jnp.logical_and(Gn >= 2, Gn != (13 if H13 else 0)))(lambda: wo_wait(Gn))
        pl.when(Gn == 6)(lambda: xb_copy().wait())

    def halves(G):
        def qp(h):
            def before(k):
                if HFIRST:
                    if k == 1:
                        wq_piece_start(G + 3, 4 * h, 8)
                    if k == 0:
                        return
                wq_piece_start(G + 3, 4 * h + k, 8)
            qproj(G + 2, h * HM, HM, before=before)
        if HFIRST:
            qp(0)
        attn_units(G, 0, 4)
        if not HFIRST:
            qp(0)
        for c in start_copies(G, 1):
            c.wait()
        wo01(G).wait()
        if HFIRST:
            qp(1)
        attn_units(G, 4, 8)
        if not HFIRST:
            qp(1)
        oproj_t(G)
        wait_top(G + 1)

    def full(G):
        n = M // QSPLIT
        def qp(t):
            def before(k):
                if QFIRST and t == 0:
                    if k == 1:
                        wq_piece_start(G + 3, 0, 4 * QSPLIT)
                    if k == 0:
                        return
                wq_piece_start(G + 3, 4 * t + k, 4 * QSPLIT)
            qproj(G + 2, n * t, n, before=before)
        if QFIRST:
            qp(0)
        a_transpose(jnp.clip(G - 8, 0, 6))
        attn_units(G, 0, 8, do_refill=True)
        for t in range(QFIRST, QSPLIT):
            qp(t)
        oproj_t(G)
        wait_top(G + 1)

    def body_h(G, carry):
        halves(G)
        return carry

    def body_f(G, carry):
        full(G)
        return carry

    lax.fori_loop(0, 2, body_h, 0)
    lax.fori_loop(2, NLOOP, body_f, 0)

    for h in range(2):
        for u in range(4 * h, 4 * h + 4):
            o2 = attn_unit(1, 2, 6, u, u * SQ, before=pins15(0, 4)(u) if h == 1 else None)
            o_s[u * SQ:(u + 1) * SQ, 0:DH] = o2[0]
            o_s[u * SQ:(u + 1) * SQ, DH:GW] = o2[1]
        if h == 0:
            a_transpose(6)
            bulk_wait_h(14, 1)
    oproj_t(14)
    for c in last_copies(0):
        c.wait()
    piece15_wait(0)
    wo_wait(15)

    for k in range(3):
        b0, nb = T2[k]
        if k < 2:
            tt = jnp.concatenate([acct_s[3 * k + j, 384:, :].T for j in range(4)], axis=0)[64 * k:64 * k + HM]
        if k == 1:
            acc2_s[...] = tt[3 * SQ:]
        os_ = [jnp.concatenate(attn_unit(1, 3, 7, u, u * SQ, before=pins15(k + 1, b0)(u) if k < 2 else None), axis=1)
               for u in range(b0, b0 + nb)]
        for u in range(b0, b0 + nb):
            r = lax.dot_general(os_[u - b0], wo_s[15 & (NWS - 1)], NT, preferred_element_type=f32)
            t = tt[(u - b0) * SQ:(u - b0 + 1) * SQ] if k < 2 else acc2_s[...]
            ob_s[u * SQ:(u + 1) * SQ, 384:896] = (t + r).astype(bf16)
        out_copy(k).start()
        if k == 1:
            out_copy(3).start()
        if k < 2:
            for c in last_copies(k + 1):
                c.wait()
            piece15_wait(k + 1)
        else:
            for j in range(4):
                out_copy(j).wait()


@jax.jit
def pallas_concat_heads__gqa_block_cached__mha_block_cached__near_ridge_kernel(A_x, A_k_cache, A_v_cache, A_wq, A_wo, B_x, B_k_cache, B_v_cache, B_wq, B_wo):
    hbm = pl.BlockSpec(memory_space=pl.ANY)
    out = pl.pallas_call(
        kernel,
        in_specs=[hbm] * 10,
        out_specs=hbm,
        out_shape=jax.ShapeDtypeStruct((M, 2 * D), bf16),
        scratch_shapes=[
            pltpu.VMEM((2, M, D), bf16),
            pltpu.VMEM((8, B, 2 * SK, DH), bf16),
            pltpu.VMEM((8, B, 2 * SK, DH), bf16),
            pltpu.VMEM((NWS, D, GW), bf16),
            pltpu.VMEM((NWS, 512, GW), bf16),
            pltpu.VMEM((4, M, GW), bf16),
            pltpu.VMEM((M, GW), bf16),
            pltpu.VMEM((7, 2 * D, 128), f32),
            pltpu.VMEM((SQ, 512), f32),
            pltpu.VMEM((M, 2 * D), bf16),
            pltpu.SemaphoreType.DMA((NSEM,)),
            pltpu.SemaphoreType.DMA((2,)),
            pltpu.SemaphoreType.DMA((2,)),
            pltpu.SemaphoreType.DMA((NWS,)),
            pltpu.SemaphoreType.DMA((NWS,)),
        ],
        compiler_params=pltpu.CompilerParams(vmem_limit_bytes=110 * 1024 * 1024, disable_bounds_checks=True,
                                             disable_semaphore_checks=True),
    )(A_x.reshape(M, D), A_k_cache, A_v_cache, A_wq, A_wo.T, B_x.reshape(M, D), B_k_cache.reshape(B, 16 * SK, DH), B_v_cache.reshape(B, 16 * SK, DH), B_wq, B_wo.T)
    return out.reshape(B, SQ, 2 * D)
```

```python
import jax
import jax.numpy as jnp
from jax import lax
import jax.experimental.pallas as pl
import jax.experimental.pallas.tpu as pltpu

B, SQ, D, SK, DH = 8, 112, 448, 512, 256
M = B * SQ
HM = M // 2
GW = 2 * DH
NGRP = 16
NLOOP = 14
NWS = 4
NT = (((1,), (1,)), ((), ()))
f32 = jnp.float32
bf16 = jnp.bfloat16
SCALE = DH ** -0.5
P0, P1 = 0, 1
R0 = 176
LA = 5
T2 = ((0, 4), (4, 3), (7, 1))
S_X = 0
S_B = 3
S_W0 = S_B + 64
S_OUT = S_W0 + 5
NSEM = S_OUT + 4


def _softmax_parts(s):
    m = jnp.max(s, axis=-1, keepdims=True)
    p = jnp.exp(s - m)
    l = jnp.sum(p, axis=-1, keepdims=True)
    r = pl.reciprocal(l, approx=True)
    r = r * (2.0 - l * r)
    return p.astype(bf16), r


def _shr(x, n):
    return x >> n if isinstance(x, int) else lax.shift_right_logical(x, n)


def _and(x, n):
    return x & n if isinstance(x, int) else lax.bitwise_and(x, n)


def _mult(x, n):
    return x if isinstance(x, int) else pl.multiple_of(x, n)


def _when(cond, fn):
    if isinstance(cond, bool):
        if cond:
            fn()
    else:
        pl.when(cond)(fn)


def _rng(G, lo, hi):
    if isinstance(G, int):
        return lo <= G < hi
    return jnp.logical_and(G >= lo, G < hi)


def _kernel(ax_h, ak_h, av_h, awq_h, awo_h, bx_h, bk_h, bv_h, bwq_h, bwo_h, out_h,
            x_s, k_s, v_s, wq_s, wo_s, q_s, o_s, acct_s, acc2_s, ob_s,
            sem, ksem, vsem, wqsem, wosem):
    cp = pltpu.make_async_copy
    KV = ((ak_h, bk_h, k_s, ksem), (av_h, bv_h, v_s, vsem))

    def per_branch(G, fn, hi=NGRP):
        g = _and(G, 7)
        _when(G < 8, lambda: fn(0, g))
        _when(_rng(G, 8, hi), lambda: fn(1, g))

    def piece(kind, br, g, u, j, par):
        a_h, b_h, buf, ps = KV[kind]
        if br == 0:
            h = R0 // 2
            return cp(a_h.at[u, g, pl.ds(j * h, h)], buf.at[g, u, pl.ds(j * h, h)], ps.at[par])
        r = j * (2 * SK - R0)
        return cp(b_h.at[u, pl.ds(_mult(2 * SK * g + r, 16), R0)], buf.at[g, u, pl.ds(r, R0)], ps.at[par])

    def piece_wait(br, g, u0, nu, par):
        for kind in range(2):
            for r in ((0,), (0, 2 * SK - R0))[br]:
                dst = KV[kind][2].at[g, pl.ds(u0, nu), pl.ds(r, R0)]
                cp(dst, dst, KV[kind][3].at[par]).wait()

    def pins(start, first):
        def before(kind, j):
            if first and kind == 0:
                if j == 1:
                    start(0, 0)
                    start(0, 1)
            else:
                start(kind, j)
        return before

    def bulk(br, g, b0, nb, r0, s):
        out = []
        for a_h, b_h, buf, _ in KV:
            if br == 0:
                out.append(cp(a_h.at[pl.ds(b0, nb), g, pl.ds(r0, SK - r0)],
                              buf.at[g, pl.ds(b0, nb), pl.ds(r0, SK - r0)], sem.at[s]))
            else:
                n = 2 * (SK - r0)
                out.append(cp(b_h.at[pl.ds(b0, nb), pl.ds(_mult(2 * SK * g + r0, 16), n)],
                              buf.at[g, pl.ds(b0, nb), pl.ds(r0, n)], sem.at[s]))
        return out

    def bulk_group(br, G):
        return bulk(br, _and(G, 7), 0, B, R0, S_B + 4 * G)

    def bulk_half(br, G, h, r0=R0):
        return bulk(br, _and(G, 7), 4 * h, 4, r0, S_B + 4 * G + h)

    def bulk_last(k):
        return bulk(1, 7, T2[k][0], T2[k][1], R0, S_B + 60 + k)

    def start_all(copies, priority=P1):
        for c in copies:
            c.start(priority=priority)

    def wait_all(copies):
        for c in copies:
            c.wait()

    def refill(G):
        Gn = G + LA
        pl.when(_rng(Gn, 8, 14))(lambda: start_all(bulk_group(1, Gn)))
        pl.when(Gn == 14)(lambda: start_all(bulk_half(1, 14, 0) + bulk_half(1, 14, 1)))
        pl.when(Gn == 15)(lambda: start_all(bulk_last(0) + bulk_last(1) + bulk_last(2)))

    def wq_copy(br, g, slot, r0, n, s):
        src = awq_h if br == 0 else bwq_h
        return cp(src.at[pl.ds(r0, n), pl.ds(_mult(g * GW, GW), GW)], wq_s.at[slot, pl.ds(r0, n)], s)

    def wo_copy(br, g, slot, r0, n, s):
        src = awo_h if br == 0 else bwo_h
        return cp(src.at[pl.ds(r0, n), pl.ds(_mult(g * GW, GW), GW)], wo_s.at[slot, pl.ds(64 + r0, n)], s)

    def wq_piece_start(G, k):
        sl = _and(G, NWS - 1)
        per_branch(G, lambda br, g: wq_copy(br, g, sl, 56 * k, 56, wqsem.at[sl]).start(priority=P0))

    def wo_piece_start(G, k):
        sl = _and(G, NWS - 1)
        per_branch(G, lambda br, g: wo_copy(br, g, sl, 32 * k, 32, wosem.at[sl]).start(priority=P0))

    def wq_wait(G):
        sl = _and(G, NWS - 1)
        wq_copy(0, 0, sl, 0, D, wqsem.at[sl]).wait()

    def wo_wait(G):
        sl = _and(G, NWS - 1)
        wo_copy(0, 0, sl, 0, D, wosem.at[sl]).wait()

    def wq_first(G):
        return wq_copy(0, G, G, 0, D, sem.at[S_W0 + G])

    def wo_first(G):
        return wo_copy(0, G, G, 0, D, sem.at[S_W0 + 3 + G])

    def xa_copy(h):
        return cp(ax_h.at[pl.ds(h * HM, HM)], x_s.at[0, pl.ds(h * HM, HM)], sem.at[S_X + h])

    def xb_copy():
        return cp(bx_h, x_s.at[1], sem.at[S_X + 2])

    def out_copy(k):
        if k < 2:
            rows, cols = pl.ds(T2[k][0] * SQ, T2[k][1] * SQ), pl.ds(0, 2 * D)
        else:
            rows, cols = pl.ds(7 * SQ, SQ), (pl.ds(384, 512) if k == 2 else pl.ds(0, 384))
        return cp(ob_s.at[rows, cols], out_h.at[rows, cols], sem.at[S_OUT + k])

    def qproj(G, r0, n, stream=None, head=False):
        x = x_s[_shr(G, 3), r0:r0 + n, :]
        for k in range(4):
            if stream is not None:
                if head and k == 1:
                    wq_piece_start(G + 1, stream)
                if not (head and k == 0):
                    wq_piece_start(G + 1, stream + k)
            q = jnp.dot(x, wq_s[_and(G, NWS - 1), :, 128 * k:128 * (k + 1)], preferred_element_type=f32)
            q_s[_and(G, NWS - 1), r0:r0 + n, 128 * k:128 * (k + 1)] = (q * SCALE).astype(bf16)

    def attn_unit(G, u, before=None):
        st = _shr(G, 3)
        r0 = u * SQ
        tile = [pl.ds(_mult(j * st * SK, SK), SK) for j in range(2)]
        s2 = []
        for j in range(2):
            if before is not None:
                before(0, j)
            s2.append(lax.dot_general(q_s[_and(G, NWS - 1), r0:r0 + SQ, j * DH:(j + 1) * DH],
                                      k_s[_and(G, 7), u, tile[j]], NT, preferred_element_type=f32))
        out = []
        for j in range(2):
            p, r = _softmax_parts(s2[j])
            if before is not None:
                before(1, j)
            o = jnp.dot(p, v_s[_and(G, 7), u, tile[j]], preferred_element_type=f32) * r
            out.append(o.astype(bf16))
        return out

    def attn_store(G, u, before=None):
        o2 = attn_unit(G, u, before)
        o_s[u * SQ:(u + 1) * SQ, 0:DH] = o2[0]
        o_s[u * SQ:(u + 1) * SQ, DH:GW] = o2[1]

    def oproj_t(G):
        c0 = _shr(G, 3) * D
        for j in range(7):
            for t in range(2):
                r = lax.dot_general(wo_s[_and(G, NWS - 1), 64 + 224 * t:64 + 224 * (t + 1), :],
                                    o_s[128 * j:128 * (j + 1), :], NT, preferred_element_type=f32)
                acct_s[j, pl.ds(_mult(c0 + 224 * t, 32), 224), :] += r
                wo_piece_start(G + 2, 2 * j + t)

    def a_transpose(j):
        ob_s[pl.ds(_mult(j * 128, 128), 128), 0:384] = acct_s[j, 0:384, :].T.astype(bf16)

    first = [wq_first(0), xa_copy(0), xa_copy(1), wq_first(1)]
    first += bulk_half(0, 0, 0, 0) + [wq_first(2)] + bulk_half(0, 0, 1) + [wo_first(0)]
    first += bulk_half(0, 1, 0) + bulk_half(0, 1, 1) + [wo_first(1)]
    first += bulk_half(0, 2, 0) + bulk_half(0, 2, 1, 0)
    for G in range(3, 8):
        if G == 5:
            first.append(xb_copy())
        first += bulk_group(0, G)
    start_all(first)
    acct_s[...] = jnp.zeros(acct_s.shape, f32)
    wo_s[15 & (NWS - 1), 0:64, :] = jnp.zeros((64, GW), bf16)
    xa_copy(0).wait()
    wq_first(0).wait()
    qproj(0, 0, HM)
    xa_copy(1).wait()
    wq_first(1).wait()
    qproj(0, HM, HM)
    qproj(1, 0, M)
    wait_all(bulk_half(0, 0, 0, 0))
    wq_first(2).wait()

    def body_halves(G, carry):
        for u in range(4):
            attn_store(G, u, pins(lambda kind, j: piece(kind, 0, G, u + 4, j, 0).start(priority=P0), u == 0))
        qproj(G + 2, 0, HM, stream=0)
        wait_all(bulk_half(0, G, 1))
        piece_wait(0, G, 4, 4, 0)
        wo_first(G).wait()
        qproj(G + 2, HM, HM, stream=4, head=True)
        for u in range(4, 8):
            attn_store(G, u, pins(lambda kind, j: piece(kind, 0, G + 1, u - 4, j, 1).start(priority=P0), u == 4))
        oproj_t(G)
        wait_all(bulk_half(0, G + 1, 0))
        piece_wait(0, G + 1, 0, 4, 1)
        wq_wait(G + 3)

        @pl.when(G == 1)
        def _():
            wait_all(bulk_half(0, 2, 1, 0))
            wo_wait(2)
        return carry

    lax.fori_loop(0, 2, body_halves, 0)

    def body_full(G, carry):
        Gn = G + 1
        qproj(G + 2, 0, HM, stream=0, head=True)
        a_transpose(jnp.clip(G - 8, 0, 6))
        for u in range(B):
            def start(kind, j):
                per_branch(Gn, lambda br, g: piece(kind, br, g, u, j, _and(Gn, 1)).start(priority=P0))
            attn_store(G, u, pins(start, u == 0))
            if u == 1:
                refill(G)
        qproj(G + 2, HM, HM, stream=4)
        oproj_t(G)
        per_branch(Gn, lambda br, g: piece_wait(br, g, 0, B, _and(Gn, 1)))
        per_branch(Gn, lambda br, g: wait_all(bulk_group(br, Gn)), hi=14)
        pl.when(Gn == 14)(lambda: wait_all(bulk_half(1, 14, 0)))
        pl.when(Gn < NLOOP)(lambda: wq_wait(Gn + 2))
        wo_wait(Gn)
        pl.when(Gn == 6)(lambda: xb_copy().wait())
        return carry

    lax.fori_loop(2, NLOOP, body_full, 0)

    def pins15(k, u, first):
        i = u - first
        if i >= T2[k][1]:
            return None
        return pins(lambda kind, j: piece(kind, 1, 7, T2[k][0] + i, j, (k + 1) % 2).start(priority=P0), i == 0)

    def wait15(k):
        wait_all(bulk_last(k))
        piece_wait(1, 7, T2[k][0], T2[k][1], (k + 1) % 2)

    for u in range(4):
        attn_store(14, u)
    a_transpose(6)
    wait_all(bulk_half(1, 14, 1))
    for u in range(4, 8):
        attn_store(14, u, pins15(0, u, 4))
    oproj_t(14)
    wait15(0)
    wo_wait(15)

    for k in range(3):
        b0, nb = T2[k]
        if k < 2:
            tt = jnp.concatenate([acct_s[3 * k + j, 384:, :].T for j in range(4)], axis=0)[64 * k:64 * k + HM]
        if k == 1:
            acc2_s[...] = tt[3 * SQ:]
        os_ = [jnp.concatenate(attn_unit(15, u, pins15(k + 1, u, b0) if k < 2 else None), axis=1)
               for u in range(b0, b0 + nb)]
        for u in range(b0, b0 + nb):
            r = lax.dot_general(os_[u - b0], wo_s[15 & (NWS - 1)], NT, preferred_element_type=f32)
            t = tt[(u - b0) * SQ:(u - b0 + 1) * SQ] if k < 2 else acc2_s[...]
            ob_s[u * SQ:(u + 1) * SQ, 384:896] = (t + r).astype(bf16)
        out_copy(k).start()
        if k == 1:
            out_copy(3).start()
        if k < 2:
            wait15(k + 1)
    for k in range(4):
        out_copy(k).wait()


@jax.jit
def pallas_concat_heads__gqa_block_cached__mha_block_cached__near_ridge_kernel(
        A_x, A_k_cache, A_v_cache, A_wq, A_wo, B_x, B_k_cache, B_v_cache, B_wq, B_wo):
    hbm = pl.BlockSpec(memory_space=pl.ANY)
    out = pl.pallas_call(
        _kernel,
        in_specs=[hbm] * 10,
        out_specs=hbm,
        out_shape=jax.ShapeDtypeStruct((M, 2 * D), bf16),
        scratch_shapes=[
            pltpu.VMEM((2, M, D), bf16),
            pltpu.VMEM((8, B, 2 * SK, DH), bf16),
            pltpu.VMEM((8, B, 2 * SK, DH), bf16),
            pltpu.VMEM((NWS, D, GW), bf16),
            pltpu.VMEM((NWS, 512, GW), bf16),
            pltpu.VMEM((NWS, M, GW), bf16),
            pltpu.VMEM((M, GW), bf16),
            pltpu.VMEM((7, 2 * D, 128), f32),
            pltpu.VMEM((SQ, 512), f32),
            pltpu.VMEM((M, 2 * D), bf16),
            pltpu.SemaphoreType.DMA((NSEM,)),
            pltpu.SemaphoreType.DMA((2,)),
            pltpu.SemaphoreType.DMA((2,)),
            pltpu.SemaphoreType.DMA((NWS,)),
            pltpu.SemaphoreType.DMA((NWS,)),
        ],
        compiler_params=pltpu.CompilerParams(
            vmem_limit_bytes=110 * 1024 * 1024,
            disable_bounds_checks=True,
            disable_semaphore_checks=True),
    )(A_x.reshape(M, D), A_k_cache, A_v_cache, A_wq, A_wo.T,
      B_x.reshape(M, D), B_k_cache.reshape(B, 16 * SK, DH), B_v_cache.reshape(B, 16 * SK, DH),
      B_wq, B_wo.T)
    return out.reshape(B, SQ, 2 * D)
```

```python
import jax
import jax.numpy as jnp
from jax import lax
import jax.experimental.pallas as pl
import jax.experimental.pallas.tpu as pltpu

B, SQ, D, SK, DH = 8, 112, 448, 512, 256
M = B * SQ
HM = M // 2
GW = 2 * DH
NGRP = 16
NLOOP = 14
NWS = 4
NT = (((1,), (1,)), ((), ()))
f32 = jnp.float32
bf16 = jnp.bfloat16
SCALE = DH ** -0.5
P0, P1 = 0, 1
R0 = 176
LA = 5
XC = ((0, 448), (448, 112), (560, 336))
T2 = ((0, 4), (4, 3), (7, 1))
S_X = 0
S_B = 5
S_W0 = S_B + 64
S_OUT = S_W0 + 5
NSEM = S_OUT + 4


def _softmax_parts(s):
    m = jnp.max(s, axis=-1, keepdims=True)
    p = jnp.exp(s - m)
    l = jnp.sum(p, axis=-1, keepdims=True)
    r = pl.reciprocal(l, approx=True)
    r = r * (2.0 - l * r)
    return p.astype(bf16), r


def _shr(x, n):
    return x >> n if isinstance(x, int) else lax.shift_right_logical(x, n)


def _and(x, n):
    return x & n if isinstance(x, int) else lax.bitwise_and(x, n)


def _mult(x, n):
    return x if isinstance(x, int) else pl.multiple_of(x, n)


def _when(cond, fn):
    if isinstance(cond, bool):
        if cond:
            fn()
    else:
        pl.when(cond)(fn)


def _rng(G, lo, hi):
    if isinstance(G, int):
        return lo <= G < hi
    return jnp.logical_and(G >= lo, G < hi)


def _kernel(ax_h, ak_h, av_h, awq_h, awo_h, bx_h, bk_h, bv_h, bwq_h, bwo_h, out_h,
            x_s, k_s, v_s, wq_s, wo_s, q_s, o_s, acct_s, acc2_s, ob_s,
            sem, ksem, vsem, wqsem, wosem):
    cp = pltpu.make_async_copy
    KV = ((ak_h, bk_h, k_s, ksem), (av_h, bv_h, v_s, vsem))

    def per_branch(G, fn, hi=NGRP):
        g = _and(G, 7)
        _when(G < 8, lambda: fn(0, g))
        _when(_rng(G, 8, hi), lambda: fn(1, g))

    def piece(kind, br, g, u, j, par):
        a_h, b_h, buf, ps = KV[kind]
        if br == 0:
            h = R0 // 2
            return cp(a_h.at[u, g, pl.ds(j * h, h)], buf.at[g, u, pl.ds(j * h, h)], ps.at[par])
        r = j * (2 * SK - R0)
        return cp(b_h.at[u, pl.ds(_mult(2 * SK * g + r, 16), R0)], buf.at[g, u, pl.ds(r, R0)], ps.at[par])

    def piece_wait(br, g, u0, nu, par):
        for kind in range(2):
            for r in ((0,), (0, 2 * SK - R0))[br]:
                dst = KV[kind][2].at[g, pl.ds(u0, nu), pl.ds(r, R0)]
                cp(dst, dst, KV[kind][3].at[par]).wait()

    def pins(start, first):
        def before(kind, j):
            if first and kind == 0:
                if j == 1:
                    start(0, 0)
                    start(0, 1)
            else:
                start(kind, j)
        return before

    def bulk(br, g, b0, nb, r0, s):
        out = []
        for a_h, b_h, buf, _ in KV:
            if br == 0:
                out.append(cp(a_h.at[pl.ds(b0, nb), g, pl.ds(r0, SK - r0)],
                              buf.at[g, pl.ds(b0, nb), pl.ds(r0, SK - r0)], sem.at[s]))
            else:
                n = 2 * (SK - r0)
                out.append(cp(b_h.at[pl.ds(b0, nb), pl.ds(_mult(2 * SK * g + r0, 16), n)],
                              buf.at[g, pl.ds(b0, nb), pl.ds(r0, n)], sem.at[s]))
        return out

    def bulk_group(br, G):
        return bulk(br, _and(G, 7), 0, B, R0, S_B + 4 * G)

    def bulk_half(br, G, h, r0=R0):
        return bulk(br, _and(G, 7), 4 * h, 4, r0, S_B + 4 * G + h)

    def bulk_last(k):
        return bulk(1, 7, T2[k][0], T2[k][1], R0, S_B + 60 + k)

    def start_all(copies, priority=P1):
        for c in copies:
            c.start(priority=priority)

    def wait_all(copies):
        for c in copies:
            c.wait()

    def refill(G):
        Gn = G + LA
        pl.when(_rng(Gn, 8, 14))(lambda: start_all(bulk_group(1, Gn)))
        pl.when(Gn == 14)(lambda: start_all(bulk_half(1, 14, 0) + bulk_half(1, 14, 1)))
        pl.when(Gn == 15)(lambda: start_all(bulk_last(0) + bulk_last(1) + bulk_last(2)))

    def wq_copy(br, g, slot, r0, n, s):
        src = awq_h if br == 0 else bwq_h
        return cp(src.at[pl.ds(r0, n), pl.ds(_mult(g * GW, GW), GW)], wq_s.at[slot, pl.ds(r0, n)], s)

    def wo_copy(br, g, slot, r0, n, s):
        src = awo_h if br == 0 else bwo_h
        return cp(src.at[pl.ds(r0, n), pl.ds(_mult(g * GW, GW), GW)], wo_s.at[slot, pl.ds(64 + r0, n)], s)

    def wq_piece_start(G, k):
        sl = _and(G, NWS - 1)
        per_branch(G, lambda br, g: wq_copy(br, g, sl, 56 * k, 56, wqsem.at[sl]).start(priority=P0))

    def wo_piece_start(G, k):
        sl = _and(G, NWS - 1)
        per_branch(G, lambda br, g: wo_copy(br, g, sl, 32 * k, 32, wosem.at[sl]).start(priority=P0))

    def wq_wait(G):
        sl = _and(G, NWS - 1)
        wq_copy(0, 0, sl, 0, D, wqsem.at[sl]).wait()

    def wo_wait(G):
        sl = _and(G, NWS - 1)
        wo_copy(0, 0, sl, 0, D, wosem.at[sl]).wait()

    def wq_first(G):
        return wq_copy(0, G, G, 0, D, sem.at[S_W0 + G])

    def wo_first(G):
        return wo_copy(0, G, G, 0, D, sem.at[S_W0 + 3 + G])

    def xa_copy(h):
        r0, n = XC[h]
        return cp(ax_h.at[pl.ds(r0, n)], x_s.at[0, pl.ds(r0, n)], sem.at[S_X + h])

    def xb_copy():
        return cp(bx_h, x_s.at[1], sem.at[S_X + 3])

    def wq0_half(h):
        return cp(awq_h.at[:, pl.ds(h * DH, DH)], wq_s.at[0, :, pl.ds(h * DH, DH)],
                  sem.at[S_W0 if h == 0 else S_X + 4])

    def out_copy(k):
        if k < 2:
            rows, cols = pl.ds(T2[k][0] * SQ, T2[k][1] * SQ), pl.ds(0, 2 * D)
        else:
            rows, cols = pl.ds(7 * SQ, SQ), (pl.ds(384, 512) if k == 2 else pl.ds(0, 384))
        return cp(ob_s.at[rows, cols], out_h.at[rows, cols], sem.at[S_OUT + k])

    def qproj(G, r0, n, stream=None, head=False, ks=range(4)):
        x = x_s[_shr(G, 3), r0:r0 + n, :]
        for k in ks:
            if stream is not None:
                if head and k == 1:
                    wq_piece_start(G + 1, stream)
                if not (head and k == 0):
                    wq_piece_start(G + 1, stream + k)
            q = jnp.dot(x, wq_s[_and(G, NWS - 1), :, 128 * k:128 * (k + 1)], preferred_element_type=f32)
            q_s[_and(G, NWS - 1), r0:r0 + n, 128 * k:128 * (k + 1)] = (q * SCALE).astype(bf16)

    def attn_unit(G, u, before=None):
        st = _shr(G, 3)
        r0 = u * SQ
        tile = [pl.ds(_mult(j * st * SK, SK), SK) for j in range(2)]
        s2 = []
        for j in range(2):
            if before is not None:
                before(0, j)
            s2.append(lax.dot_general(q_s[_and(G, NWS - 1), r0:r0 + SQ, j * DH:(j + 1) * DH],
                                      k_s[_and(G, 7), u, tile[j]], NT, preferred_element_type=f32))
        out = []
        for j in range(2):
            p, r = _softmax_parts(s2[j])
            if before is not None:
                before(1, j)
            o = jnp.dot(p, v_s[_and(G, 7), u, tile[j]], preferred_element_type=f32) * r
            out.append(o.astype(bf16))
        return out

    def attn_store(G, u, before=None):
        o2 = attn_unit(G, u, before)
        o_s[u * SQ:(u + 1) * SQ, 0:DH] = o2[0]
        o_s[u * SQ:(u + 1) * SQ, DH:GW] = o2[1]

    def oproj_t(G):
        c0 = _shr(G, 3) * D
        for j in range(7):
            for t in range(2):
                r = lax.dot_general(wo_s[_and(G, NWS - 1), 64 + 224 * t:64 + 224 * (t + 1), :],
                                    o_s[128 * j:128 * (j + 1), :], NT, preferred_element_type=f32)
                acct_s[j, pl.ds(_mult(c0 + 224 * t, 32), 224), :] += r
                wo_piece_start(G + 2, 2 * j + t)

    def a_transpose(j):
        ob_s[pl.ds(_mult(j * 128, 128), 128), 0:384] = acct_s[j, 0:384, :].T.astype(bf16)

    first = [wq0_half(0), xa_copy(0), wq0_half(1), xa_copy(1), xa_copy(2), wq_first(1)]
    first += bulk_half(0, 0, 0, 0) + [wq_first(2)] + bulk_half(0, 0, 1) + [wo_first(0)]
    first += bulk_half(0, 1, 0) + bulk_half(0, 1, 1) + [wo_first(1)]
    first += bulk_half(0, 2, 0) + bulk_half(0, 2, 1, 0)
    first.append(xb_copy())
    for G in range(3, 8):
        first += bulk_group(0, G)
    start_all(first)
    acct_s[...] = jnp.zeros(acct_s.shape, f32)
    wo_s[15 & (NWS - 1), 0:64, :] = jnp.zeros((64, GW), bf16)
    xa_copy(0).wait()
    wq0_half(0).wait()
    qproj(0, *XC[0], ks=(0, 1))
    wq0_half(1).wait()
    xa_copy(1).wait()
    qproj(0, *XC[0], ks=(2, 3))
    qproj(0, *XC[1])
    xa_copy(2).wait()
    wq_first(1).wait()
    qproj(0, *XC[2])
    qproj(1, 0, M)
    wait_all(bulk_half(0, 0, 0, 0))
    wq_first(2).wait()

    def body_halves(G, carry):
        for u in range(4):
            attn_store(G, u, pins(lambda kind, j: piece(kind, 0, G, u + 4, j, 0).start(priority=P0), u == 0))
        qproj(G + 2, 0, HM, stream=0)
        wait_all(bulk_half(0, G, 1))
        piece_wait(0, G, 4, 4, 0)
        wo_first(G).wait()
        qproj(G + 2, HM, HM, stream=4, head=True)
        for u in range(4, 8):
            attn_store(G, u, pins(lambda kind, j: piece(kind, 0, G + 1, u - 4, j, 1).start(priority=P0), u == 4))
        oproj_t(G)
        wait_all(bulk_half(0, G + 1, 0))
        piece_wait(0, G + 1, 0, 4, 1)
        wq_wait(G + 3)

        @pl.when(G == 1)
        def _():
            wait_all(bulk_half(0, 2, 1, 0))
            wo_wait(2)
            xb_copy().wait()
        return carry

    lax.fori_loop(0, 2, body_halves, 0)

    def body_full(G, carry):
        Gn = G + 1
        gn, parn, sbn = _and(Gn, 7), _and(Gn, 1), S_B + 4 * Gn
        is_a, is_b, has_q = Gn < 8, Gn >= 8, Gn < NLOOP
        is_b_full, not_b_full = _rng(Gn, 8, 14), jnp.logical_or(Gn < 8, Gn >= 14)
        qproj(G + 2, 0, HM, stream=0, head=True)
        a_transpose(jnp.clip(G - 8, 0, 6))
        for u in range(B):
            def start(kind, j):
                per_branch(Gn, lambda br, g: piece(kind, br, g, u, j, _and(Gn, 1)).start(priority=P0))
            attn_store(G, u, pins(start, u == 0))
            if u == 1:
                refill(G)
        qproj(G + 2, HM, HM, stream=4)
        oproj_t(G)
        pl.when(is_b_full)(lambda: wait_all(bulk(1, gn, 0, B, R0, sbn)))
        pl.when(not_b_full)(lambda: wait_all(bulk(0, gn, 0, B, R0, sbn)))
        pl.when(is_b)(lambda: piece_wait(1, gn, 0, B, parn))
        pl.when(is_a)(lambda: piece_wait(0, gn, 0, B, parn))
        wo_wait(Gn)
        pl.when(has_q)(lambda: wq_wait(Gn + 2))
        return carry

    lax.fori_loop(2, NLOOP, body_full, 0)

    def pins15(k, u, first):
        i = u - first
        if i >= T2[k][1]:
            return None
        return pins(lambda kind, j: piece(kind, 1, 7, T2[k][0] + i, j, (k + 1) % 2).start(priority=P0), i == 0)

    def wait15(k):
        wait_all(bulk_last(k))
        piece_wait(1, 7, T2[k][0], T2[k][1], (k + 1) % 2)

    for u in range(4):
        attn_store(14, u)
    a_transpose(6)
    wait_all(bulk_half(1, 14, 1))
    for u in range(4, 8):
        attn_store(14, u, pins15(0, u, 4))
    oproj_t(14)
    wait15(0)
    wo_wait(15)

    for k in range(3):
        b0, nb = T2[k]
        if k < 2:
            tt = jnp.concatenate([acct_s[3 * k + j, 384:, :].T for j in range(4)], axis=0)[64 * k:64 * k + HM]
        if k == 1:
            acc2_s[...] = tt[3 * SQ:]
        os_ = [jnp.concatenate(attn_unit(15, u, pins15(k + 1, u, b0) if k < 2 else None), axis=1)
               for u in range(b0, b0 + nb)]
        for u in range(b0, b0 + nb):
            r = lax.dot_general(os_[u - b0], wo_s[15 & (NWS - 1)], NT, preferred_element_type=f32)
            t = tt[(u - b0) * SQ:(u - b0 + 1) * SQ] if k < 2 else acc2_s[...]
            ob_s[u * SQ:(u + 1) * SQ, 384:896] = (t + r).astype(bf16)
        out_copy(k).start()
        if k == 1:
            out_copy(3).start()
        if k < 2:
            wait15(k + 1)
    for k in range(4):
        out_copy(k).wait()


@jax.jit
def pallas_concat_heads__gqa_block_cached__mha_block_cached__near_ridge_kernel(
        A_x, A_k_cache, A_v_cache, A_wq, A_wo, B_x, B_k_cache, B_v_cache, B_wq, B_wo):
    hbm = pl.BlockSpec(memory_space=pl.ANY)
    out = pl.pallas_call(
        _kernel,
        in_specs=[hbm] * 10,
        out_specs=hbm,
        out_shape=jax.ShapeDtypeStruct((M, 2 * D), bf16),
        scratch_shapes=[
            pltpu.VMEM((2, M, D), bf16),
            pltpu.VMEM((8, B, 2 * SK, DH), bf16),
            pltpu.VMEM((8, B, 2 * SK, DH), bf16),
            pltpu.VMEM((NWS, D, GW), bf16),
            pltpu.VMEM((NWS, 512, GW), bf16),
            pltpu.VMEM((NWS, M, GW), bf16),
            pltpu.VMEM((M, GW), bf16),
            pltpu.VMEM((7, 2 * D, 128), f32),
            pltpu.VMEM((SQ, 512), f32),
            pltpu.VMEM((M, 2 * D), bf16),
            pltpu.SemaphoreType.DMA((NSEM,)),
            pltpu.SemaphoreType.DMA((2,)),
            pltpu.SemaphoreType.DMA((2,)),
            pltpu.SemaphoreType.DMA((NWS,)),
            pltpu.SemaphoreType.DMA((NWS,)),
        ],
        compiler_params=pltpu.CompilerParams(
            vmem_limit_bytes=110 * 1024 * 1024,
            disable_bounds_checks=True,
            disable_semaphore_checks=True),
    )(A_x.reshape(M, D), A_k_cache, A_v_cache, A_wq, A_wo.T,
      B_x.reshape(M, D), B_k_cache.reshape(B, 16 * SK, DH), B_v_cache.reshape(B, 16 * SK, DH),
      B_wq, B_wo.T)
    return out.reshape(B, SQ, 2 * D)
```
